```python
import os as _os
_os.environ.setdefault("JAX_PLATFORMS", "cpu")
import jax
import jax.numpy as jnp

def _softmax(x, axis=-1):
    return jax.nn.softmax(x, axis=axis)
def _gelu(x):
    return jax.nn.gelu(x, approximate=True)
def _silu(x):
    return jax.nn.silu(x)
def _sigmoid(x):
    return jax.nn.sigmoid(x)
def _layernorm(x, axis=-1, eps=1e-5):
    m = jnp.mean(x, axis=axis, keepdims=True)
    v = jnp.var(x, axis=axis, keepdims=True)
    return (x - m) / jnp.sqrt(v + eps)
def _scatter_add(tgt, idx, src, axis=0):
    return tgt.at[idx].add(src)
def _segment_sum(src, seg, n):
    return jax.ops.segment_sum(src, seg, n)
class _Rng:
    def __init__(self, key):
        self._k = key
    def _next(self):
        self._k, sub = jax.random.split(self._k)
        return sub
    def normal(self, shape):
        return jax.random.normal(self._next(), shape, dtype=jnp.bfloat16)
    def randint(self, lo, hi, shape):
        return jax.random.randint(self._next(), shape, lo, hi, dtype=jnp.int32)
    def uniform(self, shape, lo=0.0, hi=1.0):
        return jax.random.uniform(self._next(), shape, jnp.bfloat16, lo, hi)
    def permutation(self, n):
        return jax.random.permutation(self._next(), n)


kernel_name = 'standalone__detection_seg_fpn_lateral__vision'

def setup_inputs():
    _rng = _Rng(jax.random.key(int.from_bytes(__import__("os").urandom(4), "little")))
    _w = (lambda a: (lambda t: t.astype(jnp.bfloat16) if jnp.issubdtype(t.dtype, jnp.floating) else t)(jnp.asarray(a)))
    H = W = (256 // 2) * 2
    C = 384
    k = 1
    return {
        "c_fine": _w((lambda *s: _rng.normal(s) * 0.05)(1, H, W, C)),
        "p_coarse": _w((lambda *s: _rng.normal(s) * 0.05)(1, H // 2, W // 2, C)),
        "w_lat": _w((lambda *s: _rng.normal(s) * 0.05)(C, C)),
        "w_out": _w((lambda *s: _rng.normal(s) * 0.05)(k, k, C, C)),
    }

def reference(c_fine, p_coarse, w_lat, w_out):
    B, H, W, C = c_fine.shape
    k = 1
    lat = jnp.einsum("bhwc,cd->bhwd", c_fine, w_lat)
    up = jnp.repeat(jnp.repeat(p_coarse, 2, axis=1), 2, axis=2)
    m = lat + up
    pad = k // 2
    mp = jnp.pad(m, ((0, 0), (pad, pad), (pad, pad), (0, 0)))
    o = None
    for di in range(k):
        for dj in range(k):
            t = jnp.einsum("bhwc,cd->bhwd", mp[:, di:di + H, dj:dj + W, :], w_out[di, dj])
            o = t if o is None else o + t
    return o
```

```python
import jax
import jax.numpy as jnp
from jax import lax
import jax.experimental.pallas as pl
import jax.experimental.pallas.tpu as pltpu

_A = 16
_S = 32
_BOUNDS = (0, 1, 3, 8, 16, 24, 40, 56, 63, 64)
_X = 37
_K = 4
_R = 2


@jax.jit
def pallas_standalone__detection_seg_fpn_lateral__vision_kernel(
    c_fine: jax.Array,
    p_coarse: jax.Array,
    w_lat: jax.Array,
    w_out: jax.Array,
):
    f32, bf16 = jnp.float32, jnp.bfloat16
    B, H, W, C = c_fine.shape
    A, S, bounds, X, K, R = _A, _S, _BOUNDS, _X, _K, _R
    Hh = B * H // 2 // A
    Wb = W // S
    NU = Hh * Wb
    nch = len(bounds) - 1

    def kern(c_hbm, p_hbm, wl_hbm, wo_hbm, o_hbm, cbuf, pbuf, obuf, wl_ref, wo_ref, wf_ref, up_ref, rsem, wsem):
        def rd(k):
            lo, hi = bounds[k], bounds[k + 1]
            if lo % Wb == 0 and hi % Wb == 0:
                hs, ws = pl.ds(lo // Wb, (hi - lo) // Wb), slice(None)
            else:
                hs, ws = pl.ds(lo // Wb, 1), pl.ds(lo % Wb, hi - lo)
            return (pltpu.make_async_copy(p_hbm.at[:, hs, ws], pbuf.at[:, hs, ws], rsem.at[k]),
                    pltpu.make_async_copy(c_hbm.at[:, hs, :, ws], cbuf.at[:, hs, :, ws], rsem.at[k]))

        wcp = (pltpu.make_async_copy(wl_hbm, wl_ref, wsem.at[0]),
               pltpu.make_async_copy(wo_hbm, wo_ref, wsem.at[0]))
        for cp in wcp:
            cp.start()
        for k in range(nch):
            for cp in rd(k):
                cp.start()
        for cp in wcp:
            cp.wait()
        wf_ref[...] = jnp.dot(wl_ref[...], wo_ref[...], preferred_element_type=f32).astype(bf16)

        def issued(u):
            return jnp.where(u < X - 1, 0, jnp.minimum(u + 1, K + R * (u - (X - 1))))

        def body(u, _):
            hh, wb = u // Wb, u % Wb
            for k in range(nch):
                if bounds[k] < X or k == nch - 1:
                    @pl.when(u == bounds[k])
                    def _():
                        for cp in rd(k):
                            cp.wait()
            n = A * S // 2
            q = jnp.dot(pbuf[:, hh, wb].reshape(n, C), wo_ref[...], preferred_element_type=f32)
            for j in range(C // 128):
                up_ref[j, pl.ds(0, n, stride=2), :] = q[:, j * 128:(j + 1) * 128]
                up_ref[j, pl.ds(1, n, stride=2), :] = q[:, j * 128:(j + 1) * 128]
            upv = jnp.concatenate([up_ref[j] for j in range(C // 128)], axis=1).reshape(A, 1, S, C)
            cv = cbuf[:, hh, :, wb].reshape(A * 2 * S, C)
            o = jnp.dot(cv, wf_ref[...], preferred_element_type=f32).reshape(A, 2, S, C)
            obuf[:, hh, :, wb] = (o + upv).astype(bf16)

            @pl.when(u == X - 1)
            def _():
                for k in range(nch - 1):
                    if bounds[k] >= X:
                        for cp in rd(k):
                            cp.wait()

            def wr(v, _):
                vh, vw = v // Wb, v % Wb
                for par in range(2):
                    pltpu.make_async_copy(obuf.at[:, vh, par, vw], o_hbm.at[:, vh, par, vw], wsem.at[0]).start()

            lax.fori_loop(issued(u - 1), jnp.where(u == NU - 1, NU, issued(u)), wr, None)

        lax.fori_loop(0, NU, body, None)
        pltpu.make_async_copy(obuf, o_hbm, wsem.at[0]).wait()

    out = pl.pallas_call(
        kern,
        in_specs=[pl.BlockSpec(memory_space=pl.ANY)] * 4,
        out_specs=pl.BlockSpec(memory_space=pl.ANY),
        out_shape=jax.ShapeDtypeStruct((A, Hh, 2, Wb, S, C), bf16),
        scratch_shapes=[
            pltpu.VMEM((A, Hh, 2, Wb, S, C), bf16),
            pltpu.VMEM((A, Hh, Wb, S // 2, C), bf16),
            pltpu.VMEM((A, Hh, 2, Wb, S, C), bf16),
            pltpu.VMEM((C, C), bf16),
            pltpu.VMEM((C, C), bf16),
            pltpu.VMEM((C, C), bf16),
            pltpu.VMEM((C // 128, A * S, 128), f32),
            pltpu.SemaphoreType.DMA((nch,)),
            pltpu.SemaphoreType.DMA((1,)),
        ],
        compiler_params=pltpu.CompilerParams(vmem_limit_bytes=120 * 1024 * 1024),
        name="fpn_lateral",
    )(
        c_fine.reshape(A, Hh, 2, Wb, S, C),
        p_coarse.reshape(A, Hh, Wb, S // 2, C),
        w_lat,
        w_out.reshape(C, C),
    )
    return out.reshape(B, H, W, C)
```

```python
import jax
import jax.numpy as jnp
import jax.experimental.pallas as pl
import jax.experimental.pallas.tpu as pltpu

_HALVES = 2
_BANDS = 8
_UNIT_W = 128
_READ_W = 16
_WRITE_W = 32
_READ_UNITS = 17
_C_READS = 56
_P_READS = 12
_TAIL_READS = 2
_EARLY_READS = 60
_WEIGHT_ROWS = 48
_LANES, _SUBLANES = 128, 8


def _divmod(x, n):
    assert n & (n - 1) == 0
    return x >> (n.bit_length() - 1), x & (n - 1)


def _window(start, size):
    if not isinstance(start, int):
        start = pl.multiple_of(start, size)
    return pl.ds(start, size)


@jax.jit
def pallas_standalone__detection_seg_fpn_lateral__vision_kernel(
    c_fine: jax.Array,
    p_coarse: jax.Array,
    w_lat: jax.Array,
    w_out: jax.Array,
):
    B, H, W, C = c_fine.shape
    dtype = c_fine.dtype
    A, U = _BANDS, _UNIT_W
    rows = B * H // (2 * _HALVES * A)
    cols = W // U
    n_units = _HALVES * rows * cols
    n_batches = _HALVES * rows
    lag = n_units - n_batches + 1
    c_per_unit, p_per_unit = 4 * U // _READ_W, U // _READ_W
    c_tail = n_units * c_per_unit - _TAIL_READS
    c_ahead = c_tail - _READ_UNITS * _C_READS
    p_ahead = n_units * p_per_unit - _READ_UNITS * _P_READS
    weight_sem, write_sem = 3 * n_units, 3 * n_units + 1

    assert w_out.shape == (1, 1, C, C) and C % _LANES == 0 and C % _WEIGHT_ROWS == 0
    assert c_ahead >= c_per_unit and _C_READS >= c_per_unit
    assert p_ahead >= p_per_unit and _P_READS >= p_per_unit
    assert lag <= _READ_UNITS
    assert all((v + 1) * cols <= v + lag for v in range(n_batches))

    fine_shape = (_HALVES, A, rows * 2 * W, C)
    coarse_shape = (_HALVES, A, rows * W // 2, C)
    all_bands = slice(None)

    def locate(u):
        half, k = _divmod(u, rows * cols)
        row, col = _divmod(k, cols)
        return half, row * (2 * W) + col * U, k * (U // 2)

    def kernel(
        c_hbm, p_hbm, wl_hbm, wo_hbm, o_hbm,
        c_buf, p_buf, o_buf, wl_buf, wo_buf, wf_buf, up_buf,
    ):
        def run(sems):
            def copy(src, dst, idx, sem):
                return pltpu.make_async_copy(src.at[idx], dst.at[idx], sems.at[sem])

            def c_piece(m):
                u, k = _divmod(m, c_per_unit)
                half, x, _ = locate(u)
                dy, k = _divmod(k, c_per_unit // 2)
                dx, b = _divmod(k, 2)
                return 3 * u + dy, half, b * (A // 2), x + dy * W + dx * _READ_W

            def c_read(m):
                sem, half, band, x = c_piece(m)
                idx = (half, pl.ds(band, A // 2), _window(x, _READ_W))
                return copy(c_hbm, c_buf, idx, sem)

            def p_read(m):
                u, k = _divmod(m, p_per_unit)
                half, _, x = locate(u)
                dx, b = _divmod(k, 2)
                bands = pl.ds(b * (A // 2), A // 2)
                idx = (half, bands, _window(x + dx * _READ_W, _READ_W))
                return copy(p_hbm, p_buf, idx, 3 * u + 2)

            def start_alternating(copies, first=0):
                for i, cp in enumerate(copies, first):
                    cp.start(priority=1 - i % 2)

            def wait_inputs(u):
                half, x, xc = locate(u)
                for dy in range(2):
                    idx = (half, all_bands, _window(x + dy * W, U))
                    copy(c_hbm, c_buf, idx, 3 * u + dy).wait()
                idx = (half, all_bands, _window(xc, U // 2))
                copy(p_hbm, p_buf, idx, 3 * u + 2).wait()

            def write_batch(v):
                half, row = _divmod(v, rows)
                for x in range(0, 2 * W, _WRITE_W):
                    idx = (half, all_bands, _window(row * (2 * W) + x, _WRITE_W))
                    copy(o_buf, o_hbm, idx, write_sem).start()

            def compute(u, reads=()):
                half, x, xc = locate(u)
                n = A * U // 2
                top = jnp.dot(
                    p_buf[half, :, _window(xc, U // 2)].reshape(n, C),
                    wo_buf[...],
                    preferred_element_type=jnp.float32,
                )
                for j in range(C // _LANES):
                    for phase in range(2):
                        up_buf[j, pl.ds(phase, n, stride=2), :] = top[
                            :, j * _LANES : (j + 1) * _LANES
                        ]
                up = jnp.concatenate([up_buf[j] for j in range(C // _LANES)], axis=1)
                for dy in range(2):
                    fine = _window(x + dy * W, U)
                    c = c_buf[half, :, fine].reshape(A * U, C)
                    lo, hi = dy * len(reads) // 2, (dy + 1) * len(reads) // 2
                    start_alternating(reads[lo:hi], lo)
                    lat = jnp.dot(c, wf_buf[...], preferred_element_type=jnp.float32)
                    o_buf[half, :, fine] = (lat + up).astype(dtype).reshape(A, U, C)

            weights = [
                copy(src, dst, (pl.ds(r, _WEIGHT_ROWS),), weight_sem)
                for src, dst in ((wl_hbm, wl_buf), (wo_hbm, wo_buf))
                for r in range(0, C, _WEIGHT_ROWS)
            ]
            ahead = []
            for u in range(n_units):
                ps = range(u * p_per_unit, min((u + 1) * p_per_unit, p_ahead))
                cs = range(u * c_per_unit, min((u + 1) * c_per_unit, c_ahead))
                ahead += [p_read(m) for m in ps] + [c_read(m) for m in cs]

            for cp in weights:
                cp.start(priority=1)
            start_alternating(ahead[:_EARLY_READS])
            for cp in weights:
                cp.wait()
            wf_buf[...] = jnp.dot(
                wl_buf[...], wo_buf[...], preferred_element_type=jnp.float32
            ).astype(dtype)
            start_alternating(ahead[_EARLY_READS:], _EARLY_READS)

            @pl.loop(0, _READ_UNITS)
            def _read_phase(u):
                wait_inputs(u)
                compute(
                    u,
                    [p_read(p_ahead + u * _P_READS + i) for i in range(_P_READS)]
                    + [c_read(c_ahead + u * _C_READS + i) for i in range(_C_READS)],
                )

            for m in range(c_tail, c_tail + _TAIL_READS):
                sem, half, band, x = c_piece(m)
                for dx in range(0, _READ_W, _SUBLANES):
                    for b in range(band, band + A // 2):
                        for lane in range(0, C, _LANES):
                            tile = (pl.ds(x + dx, _SUBLANES), pl.ds(lane, _LANES))
                            copy(c_hbm, c_buf, (half, b, *tile), sem).start(priority=1)

            for v in range(_READ_UNITS - lag):
                write_batch(v)

            @pl.loop(_READ_UNITS, n_units)
            def _write_phase(u):
                wait_inputs(u)
                write_batch(u - lag)
                compute(u)

            for v in range(n_units - lag, n_batches):
                write_batch(v)
            pltpu.make_async_copy(o_buf, o_hbm, sems.at[write_sem]).wait()

        pl.run_scoped(run, pltpu.SemaphoreType.DMA((write_sem + 1,)))

    out = pl.pallas_call(
        kernel,
        in_specs=[pl.BlockSpec(memory_space=pl.ANY)] * 4,
        out_specs=pl.BlockSpec(memory_space=pl.ANY),
        out_shape=jax.ShapeDtypeStruct(fine_shape, dtype),
        scratch_shapes=[
            pltpu.VMEM(fine_shape, dtype),
            pltpu.VMEM(coarse_shape, dtype),
            pltpu.VMEM(fine_shape, dtype),
            pltpu.VMEM((C, C), dtype),
            pltpu.VMEM((C, C), dtype),
            pltpu.VMEM((C, C), dtype),
            pltpu.VMEM((C // _LANES, A * U, _LANES), jnp.float32),
        ],
        compiler_params=pltpu.CompilerParams(vmem_limit_bytes=116 * 1024 * 1024),
        name="fpn_lateral",
    )(
        c_fine.reshape(fine_shape),
        p_coarse.reshape(coarse_shape),
        w_lat,
        w_out.reshape(C, C),
    )
    return out.reshape(B, H, W, C)
```
